```python
import os as _os
_os.environ.setdefault('JAX_PLATFORMS', 'cpu')
import jax
import jax.numpy as jnp

def _softmax(x, axis=-1):
    return jax.nn.softmax(x, axis=axis)

def _gelu(x):
    return jax.nn.gelu(x, approximate=True)

def _silu(x):
    return jax.nn.silu(x)

def _sigmoid(x):
    return jax.nn.sigmoid(x)

def _layernorm(x, axis=-1, eps=1e-05):
    m = jnp.mean(x, axis=axis, keepdims=True)
    v = jnp.var(x, axis=axis, keepdims=True)
    return (x - m) / jnp.sqrt(v + eps)

def _scatter_add(tgt, idx, src, axis=0):
    return tgt.at[idx].add(src)

def _segment_sum(src, seg, n):
    return jax.ops.segment_sum(src, seg, n)

class _Rng:

    def __init__(self, key):
        self._k = key

    def _next(self):
        self._k, sub = jax.random.split(self._k)
        return sub

    def normal(self, shape):
        return jax.random.normal(self._next(), shape, dtype=jnp.bfloat16)

    def randint(self, lo, hi, shape):
        return jax.random.randint(self._next(), shape, lo, hi, dtype=jnp.int32)

    def uniform(self, shape, lo=0.0, hi=1.0):
        return jax.random.uniform(self._next(), shape, jnp.bfloat16, lo, hi)

    def permutation(self, n):
        return jax.random.permutation(self._next(), n)
kernel_name = 'adaLN_cond__sliding_local_dilated__dense_activation_relu__prompt'

def setup_inputs():
    _rng = _Rng(jax.random.key(int.from_bytes(__import__("os").urandom(4), "little")))
    _w = lambda a: (lambda t: t.astype(jnp.bfloat16) if jnp.issubdtype(t.dtype, jnp.floating) else t)(jnp.asarray(a))

    def _A_setup():
        B, S, D = (1, 2048, 576)
        return {'x': _w((lambda *s: _rng.normal(s) * 0.05)(B, S, D)), 'wqkv': _w((lambda *s: _rng.normal(s) * 0.05)(D, 3 * D)), 'wo': _w((lambda *s: _rng.normal(s) * 0.05)(D, D))}
    _A_in = _A_setup()

    def _B_setup():
        B, S, D, Dff = (1, 2048, 576, 4608)
        return {'x': _w((lambda *s: _rng.normal(s) * 0.05)(B, S, D)), 'w1': _w((lambda *s: _rng.normal(s) * 0.05)(D, Dff)), 'w2': _w((lambda *s: _rng.normal(s) * 0.05)(Dff, D))}
    _B_in = _B_setup()
    return {'A_x': _A_in['x'], 'A_wqkv': _A_in['wqkv'], 'A_wo': _A_in['wo'], 'B_x': _B_in['x'], 'B_w1': _B_in['w1'], 'B_w2': _B_in['w2'], 'c': _w((lambda *s: _rng.normal(s) * 0.05)(1, 576) * 8.0), 'w_mod': _w((lambda *s: _rng.normal(s) * 0.05)(576, 6 * 576) * 576 ** (-0.5) * 8.0)}

def reference(A_x, A_wqkv, A_wo, B_x, B_w1, B_w2, c, w_mod):

    def _A_ref(x, wqkv, wo):
        B, S, D = x.shape
        H = 32
        Dh = D // H
        W, dil = (8, 2)
        qkv = (lambda x, *d: x.transpose(*d))((x @ wqkv).reshape(B, S, 3, H, Dh), 2, 0, 3, 1, 4)
        q, k, v = (qkv[0], qkv[1], qkv[2])
        scale = Dh ** (-0.5)
        pos = jnp.arange(S)
        off = jnp.arange(W) * dil
        idx = pos[:, None] - off[None, :]
        mask = idx >= 0
        idx_c = jnp.where(mask, idx, 0).reshape(-1)
        kg = k[:, :, idx_c, :].reshape(B, H, S, W, Dh)
        vg = v[:, :, idx_c, :].reshape(B, H, S, W, Dh)
        logits = jnp.einsum('bhsd,bhswd->bhsw', q, kg) * scale
        logits = jnp.where(mask[None, None, :, :], logits, -1000000000.0)
        attn = _softmax(logits, axis=-1)
        o = jnp.einsum('bhsw,bhswd->bhsd', attn, vg)
        return (lambda x, *d: x.transpose(*d))(o, 0, 2, 1, 3).reshape(B, S, D) @ wo

    def _B_ref(x, w1, w2):
        h = jnp.einsum('bsd,df->bsf', x, w1)
        zero = jnp.zeros_like(h)
        h = jnp.maximum(h, zero)
        return jnp.einsum('bsf,fd->bsd', h, w2)
    x = A_x
    mod = (_silu(c) @ w_mod).reshape(c.shape[0], 6, 1, -1)
    sa, ca, ga, sb, cb, gb = (mod[:, 0].copy(), mod[:, 1].copy(), mod[:, 2].copy(), mod[:, 3].copy(), mod[:, 4].copy(), mod[:, 5].copy())
    h = _layernorm(x, axis=-1) * (1 + ca) + sa
    x = x + ga * _A_ref(h, A_wqkv, A_wo)
    h = _layernorm(x, axis=-1) * (1 + cb) + sb
    x = x + gb * _B_ref(h, B_w1, B_w2)
    return x
```

```python
import functools

import jax
import jax.numpy as jnp
from jax import lax
import jax.experimental.pallas as pl
import jax.experimental.pallas.tpu as pltpu

_H = 32
_W = 8
_DIL = 2
_HALO = 16
_LANES = 128


def _layernorm(x, eps=1e-05):
    m = jnp.mean(x, axis=-1, keepdims=True)
    xc = x - m
    v = jnp.mean(xc * xc, axis=-1, keepdims=True)
    return xc * lax.rsqrt(v + eps)


def _kernel(x_ref, wq_ref, wk_ref, wv_ref, wo_ref, w1_ref, w2_ref, c_ref, wmod_ref,
            o_ref, mod_ref, kbuf, vbuf, *, tm, d, dp, fc, rc, scale):
    i = pl.program_id(0)
    f32, bf16 = jnp.float32, jnp.bfloat16
    dff = w1_ref.shape[1]

    @pl.when(i == 0)
    def _():
        c = c_ref[...].astype(f32)
        sc = c * jax.nn.sigmoid(c)
        mod = jnp.dot(sc.astype(bf16), wmod_ref[...], preferred_element_type=f32)
        mod_ref[...] = jnp.zeros(mod_ref.shape, f32)
        for r in range(6):
            mod_ref[r:r + 1, :] = mod[0:1, r * d:(r + 1) * d]
        kbuf[0:_HALO, :] = jnp.zeros((_HALO, dp), f32)
        vbuf[0:_HALO, :] = jnp.zeros((_HALO, dp), f32)

    @pl.when(i > 0)
    def _():
        kbuf[0:_HALO, :] = kbuf[tm:tm + _HALO, :]
        vbuf[0:_HALO, :] = vbuf[tm:tm + _HALO, :]

    sa = mod_ref[0:1, :]
    ca = mod_ref[1:2, :]
    ga = mod_ref[2:3, :]
    sb = mod_ref[3:4, :]
    cb = mod_ref[4:5, :]
    gb = mod_ref[5:6, :]

    x = x_ref[...].astype(f32)
    h = (_layernorm(x) * (1.0 + ca) + sa).astype(bf16)

    q = jnp.dot(h, wq_ref[...], preferred_element_type=f32) * scale
    kbuf[_HALO:_HALO + tm, :] = jnp.dot(h, wk_ref[...], preferred_element_type=f32)
    vbuf[_HALO:_HALO + tm, :] = jnp.dot(h, wv_ref[...], preferred_element_type=f32)

    nlb = dp // _LANES
    outs = []
    for r0 in range(0, tm, rc):
        qc = q[r0:r0 + rc, :]
        pos = i * tm + r0 + lax.broadcasted_iota(jnp.int32, (rc, _LANES), 0)
        logits = []
        for j in range(_W):
            kc = kbuf[_HALO + r0 - _DIL * j:_HALO + r0 - _DIL * j + rc, :]
            prod = qc * kc
            s = prod[:, 0:_LANES]
            for b in range(1, nlb):
                s = s + prod[:, b * _LANES:(b + 1) * _LANES]
            s = s + pltpu.roll(s, 32, 1)
            s = s + pltpu.roll(s, 64, 1)
            s = jnp.where(pos >= _DIL * j, s, -1000000000.0)
            logits.append(s)
        m = logits[0]
        for j in range(1, _W):
            m = jnp.maximum(m, logits[j])
        es = [jnp.exp(l - m) for l in logits]
        den = es[0]
        for j in range(1, _W):
            den = den + es[j]
        inv = 1.0 / den
        acc = None
        for j in range(_W):
            p = es[j] * inv
            pw = jnp.concatenate([p] * nlb, axis=1)
            vc = vbuf[_HALO + r0 - _DIL * j:_HALO + r0 - _DIL * j + rc, :]
            acc = pw * vc if acc is None else acc + pw * vc
        outs.append(acc.astype(bf16))
    o = jnp.concatenate(outs, axis=0)

    attn = jnp.dot(o, wo_ref[...], preferred_element_type=f32)
    x1 = x + ga * attn

    h2 = (_layernorm(x1) * (1.0 + cb) + sb).astype(bf16)
    y = jnp.zeros((tm, d), f32)
    for f0 in range(0, dff, fc):
        a = jnp.dot(h2, w1_ref[:, f0:f0 + fc], preferred_element_type=f32)
        a = jnp.maximum(a, 0.0).astype(bf16)
        y = y + jnp.dot(a, w2_ref[f0:f0 + fc, :], preferred_element_type=f32)
    o_ref[...] = (x1 + gb * y).astype(o_ref.dtype)


@jax.jit
def pallas_adaLN_cond__sliding_local_dilated__dense_activation_relu__prompt_kernel(
    A_x: jax.Array,
    A_wqkv: jax.Array,
    A_wo: jax.Array,
    B_x: jax.Array,
    B_w1: jax.Array,
    B_w2: jax.Array,
    c: jax.Array,
    w_mod: jax.Array,
):
    B, S, D = A_x.shape
    assert B == 1
    H = _H
    Dh = D // H
    assert Dh * H == D
    DP = ((D + _LANES - 1) // _LANES) * _LANES
    Dff = B_w1.shape[1]
    TM = 256
    FC = 512
    RC = 32
    assert S % TM == 0 and Dff % FC == 0 and TM % RC == 0

    wqkv = A_wqkv.reshape(D, 3, H, Dh).transpose(1, 0, 3, 2).reshape(3, D, D)
    wqkv = jnp.pad(wqkv, ((0, 0), (0, 0), (0, DP - D)))
    wo = A_wo.reshape(H, Dh, D).transpose(1, 0, 2).reshape(D, D)
    wo = jnp.pad(wo, ((0, DP - D), (0, 0)))
    x = A_x.reshape(S, D)

    kern = functools.partial(_kernel, tm=TM, d=D, dp=DP, fc=FC, rc=RC, scale=float(Dh) ** -0.5)

    out = pl.pallas_call(
        kern,
        grid=(S // TM,),
        in_specs=[
            pl.BlockSpec((TM, D), lambda i: (i, 0)),
            pl.BlockSpec((None, D, DP), lambda i: (0, 0, 0)),
            pl.BlockSpec((None, D, DP), lambda i: (1, 0, 0)),
            pl.BlockSpec((None, D, DP), lambda i: (2, 0, 0)),
            pl.BlockSpec((DP, D), lambda i: (0, 0)),
            pl.BlockSpec((D, Dff), lambda i: (0, 0)),
            pl.BlockSpec((Dff, D), lambda i: (0, 0)),
            pl.BlockSpec((1, D), lambda i: (0, 0)),
            pl.BlockSpec((D, 6 * D), lambda i: (0, 0)),
        ],
        out_specs=pl.BlockSpec((TM, D), lambda i: (i, 0)),
        out_shape=jax.ShapeDtypeStruct((S, D), A_x.dtype),
        scratch_shapes=[
            pltpu.VMEM((8, D), jnp.float32),
            pltpu.VMEM((TM + _HALO, DP), jnp.float32),
            pltpu.VMEM((TM + _HALO, DP), jnp.float32),
        ],
        compiler_params=pltpu.CompilerParams(
            dimension_semantics=("arbitrary",),
            vmem_limit_bytes=100 * 1024 * 1024,
        ),
    )(x, wqkv, wqkv, wqkv, wo, B_w1, B_w2, c, w_mod)
    return out.reshape(B, S, D)
```

```python
import functools

import jax
import jax.numpy as jnp
from jax import lax
import jax.experimental.pallas as pl
import jax.experimental.pallas.tpu as pltpu

_H = 32
_W = 8
_DIL = 2
_HALO = 16
_LANES = 128


def _layernorm(x, eps=1e-05):
    m = jnp.mean(x, axis=-1, keepdims=True)
    xc = x - m
    v = jnp.mean(xc * xc, axis=-1, keepdims=True)
    return xc * lax.rsqrt(v + eps)


def _kernel(x_ref, c_ref, wqkv_hbm, wo_hbm, w1_hbm, w2_hbm, wmod_hbm,
            o_ref,
            mod_ref, kbuf, vbuf, q_s, x1n_s, h2n_s, x_s, x1_s, h2_s, y_s,
            wqkv_raw, wo_raw, wmod_raw,
            wq_p, wk_p, wv_p, wo_p, w1_ref, w2_ref, sems,
            *, nt, tm, d, dp, fc, rc, nh, attn_pos, scale):
    i = pl.program_id(0)
    f32, bf16 = jnp.float32, jnp.bfloat16
    dff = w1_ref.shape[1]
    dh = d // _H
    nlb = dp // _LANES
    hm = tm // nh
    nfc = dff // fc
    fpi = (nfc - 1) // nh
    assert fpi * nh + 1 == nfc and hm % rc == 0

    cp_wqkv = pltpu.make_async_copy(wqkv_hbm, wqkv_raw, sems.at[0])
    cp_wo = pltpu.make_async_copy(wo_hbm, wo_raw, sems.at[1])
    cp_wmod = pltpu.make_async_copy(wmod_hbm, wmod_raw, sems.at[2])

    def cp_ffn(piece):
        if isinstance(piece, int) and piece == 0:
            cols = pl.ds(0, fc)
        elif isinstance(piece, int):
            cols = pl.ds(fc + (piece - 1) * fpi * fc, fpi * fc)
        else:
            cols = pl.ds(pl.multiple_of(fc + (piece - 1) * fpi * fc, fc), fpi * fc)
        return (pltpu.make_async_copy(w1_hbm.at[:, cols], w1_ref.at[:, cols], sems.at[3 + 2 * piece]),
                pltpu.make_async_copy(w2_hbm.at[:, cols], w2_ref.at[:, cols], sems.at[4 + 2 * piece]))

    def wait_ffn(piece):
        @pl.when(i == 1)
        def _():
            for cp in cp_ffn(piece):
                cp.wait()

    def setup():
        cp_wqkv.start()
        cp_wo.start()
        cp_wmod.start()
        kbuf[0:_HALO, :] = jnp.zeros((_HALO, dp), f32)
        vbuf[0:_HALO, :] = jnp.zeros((_HALO, dp), f32)

        src = lax.broadcasted_iota(jnp.int32, (d, dp), 0)
        dst = lax.broadcasted_iota(jnp.int32, (d, dp), 1)
        perm = jnp.where((src == (dst % _H) * dh + dst // _H) & (dst < d), 1.0, 0.0).astype(bf16)
        cp_wqkv.wait()
        for piece in range(nh + 1):
            for cp in cp_ffn(piece):
                cp.start()
        wq_p[...] = jnp.dot(wqkv_raw[:, 0:d], perm, preferred_element_type=f32).astype(bf16)
        wk_p[...] = jnp.dot(wqkv_raw[:, d:2 * d], perm, preferred_element_type=f32).astype(bf16)
        wv_p[...] = jnp.dot(wqkv_raw[:, 2 * d:3 * d], perm, preferred_element_type=f32).astype(bf16)
        dst_t = lax.broadcasted_iota(jnp.int32, (dp, d), 0)
        src_t = lax.broadcasted_iota(jnp.int32, (dp, d), 1)
        perm_t = jnp.where((src_t == (dst_t % _H) * dh + dst_t // _H) & (dst_t < d), 1.0, 0.0).astype(bf16)
        cp_wo.wait()
        wo_p[...] = jnp.dot(perm_t, wo_raw[...], preferred_element_type=f32).astype(bf16)

        cp_wmod.wait()
        c = c_ref[...].astype(f32)
        sc = c * jax.nn.sigmoid(c)
        mod = jnp.dot(sc.astype(bf16), wmod_raw[...], preferred_element_type=f32)
        mod_ref[...] = jnp.zeros(mod_ref.shape, f32)
        for r in range(6):
            mod_ref[r:r + 1, :] = mod[0:1, r * d:(r + 1) * d]

    def attn_pre(first):
        sa = mod_ref[0:1, :]
        ca = mod_ref[1:2, :]
        if not first:
            kbuf[0:_HALO, :] = kbuf[tm:tm + _HALO, :]
            vbuf[0:_HALO, :] = vbuf[tm:tm + _HALO, :]
        x = x_ref[...].astype(f32).T
        x_s[...] = x
        h = (_layernorm(x) * (1.0 + ca) + sa).astype(bf16)
        q_s[...] = jnp.dot(h, wq_p[...], preferred_element_type=f32) * scale
        kbuf[_HALO:_HALO + tm, :] = jnp.dot(h, wk_p[...], preferred_element_type=f32)
        vbuf[_HALO:_HALO + tm, :] = jnp.dot(h, wv_p[...], preferred_element_type=f32)

    def attn_rows(r0, first):
        qc = q_s[pl.ds(r0, rc), :]
        kwin = kbuf[pl.ds(r0, rc + _HALO), :]
        vwin = vbuf[pl.ds(r0, rc + _HALO), :]
        logits = []
        for j in range(_W):
            o0 = _HALO - _DIL * j
            prod = qc * kwin[o0:o0 + rc, :]
            s = prod[:, 0:_LANES]
            for b in range(1, nlb):
                s = s + prod[:, b * _LANES:(b + 1) * _LANES]
            s = s + pltpu.roll(s, 32, 1)
            s = s + pltpu.roll(s, 64, 1)
            if first:
                pos = r0 + lax.broadcasted_iota(jnp.int32, (rc, _LANES), 0)
                s = jnp.where(pos >= _DIL * j, s, -1000000000.0)
            logits.append(s)
        m = logits[0]
        for j in range(1, _W):
            m = jnp.maximum(m, logits[j])
        es = [jnp.exp(l - m) for l in logits]
        den = es[0]
        for j in range(1, _W):
            den = den + es[j]
        inv = 1.0 / den
        acc = None
        for j in range(_W):
            o0 = _HALO - _DIL * j
            t = jnp.concatenate([es[j]] * nlb, axis=1) * vwin[o0:o0 + rc, :]
            acc = t if acc is None else acc + t
        return (acc * jnp.concatenate([inv] * nlb, axis=1)).astype(bf16)

    def attn_block(c, first):
        ga = mod_ref[2:3, :]
        sb = mod_ref[3:4, :]
        cb = mod_ref[4:5, :]
        base = c * hm
        oa = jnp.concatenate(
            [attn_rows(pl.multiple_of(base + r, rc), first) for r in range(0, hm, rc)], axis=0)
        attn = jnp.dot(oa, wo_p[...], preferred_element_type=f32)
        rows = pl.ds(pl.multiple_of(base, hm), hm)
        x1 = x_s[rows, :] + ga * attn
        x1n_s[rows, :] = x1
        h2n_s[rows, :] = (_layernorm(x1) * (1.0 + cb) + sb).astype(bf16)

    def ffn_chunk(c):
        f0 = c * fc if isinstance(c, int) else pl.multiple_of(c * fc, fc)
        a = jnp.dot(h2_s[...], w1_ref[:, pl.ds(f0, fc)], preferred_element_type=f32)
        a = jnp.maximum(a, 0.0).astype(bf16)
        return lax.dot_general(a, w2_ref[:, pl.ds(f0, fc)], (((1,), (1,)), ((), ())),
                               preferred_element_type=f32)

    def step(do_attn, do_ffn, first):
        if do_ffn:
            x1_s[...] = x1n_s[...]
            h2_s[...] = h2n_s[...]
            wait_ffn(0)
            y_s[...] = ffn_chunk(0)
        if do_attn:
            attn_pre(first)

        def body(c, carry):
            if do_ffn:
                wait_ffn(c + 1)
            acc = None
            for k in range(fpi):
                if k == attn_pos and do_attn:
                    attn_block(c, first)
                if do_ffn:
                    t = ffn_chunk(c * fpi + 1 + k)
                    acc = t if acc is None else acc + t
            if do_ffn:
                y_s[...] += acc
            return carry

        lax.fori_loop(0, nh, body, 0)
        if do_ffn:
            gb = mod_ref[5:6, :]
            o_ref[...] = (x1_s[...] + gb * y_s[...]).T.astype(o_ref.dtype)

    @pl.when(i == 0)
    def _():
        setup()
        step(True, False, True)

    @pl.when(jnp.logical_and(i > 0, i < nt))
    def _():
        step(True, True, False)

    @pl.when(i == nt)
    def _():
        step(False, True, False)


@jax.jit
def pallas_adaLN_cond__sliding_local_dilated__dense_activation_relu__prompt_kernel(
    A_x: jax.Array,
    A_wqkv: jax.Array,
    A_wo: jax.Array,
    B_x: jax.Array,
    B_w1: jax.Array,
    B_w2: jax.Array,
    c: jax.Array,
    w_mod: jax.Array,
):
    B, S, D = A_x.shape
    assert B == 1
    H = _H
    Dh = D // H
    assert Dh * H == D
    DP = ((D + _LANES - 1) // _LANES) * _LANES
    Dff = B_w1.shape[1]
    TM = 256
    FC = 512
    RC = 32
    NH = 2
    assert S % TM == 0 and Dff % FC == 0 and S // TM >= 2
    NT = S // TM

    x = A_x.reshape(S, D).T
    w2t = B_w2.T
    bf16 = jnp.bfloat16
    f32 = jnp.float32

    kern = functools.partial(_kernel, nt=NT, tm=TM, d=D, dp=DP, fc=FC, rc=RC, nh=NH,
                             attn_pos=2, scale=float(Dh) ** -0.5)
    hbm = pl.BlockSpec(memory_space=pl.ANY)

    out = pl.pallas_call(
        kern,
        grid=(NT + 1,),
        in_specs=[
            pl.BlockSpec((D, TM), lambda i: (0, jnp.minimum(i, NT - 1))),
            pl.BlockSpec((1, D), lambda i: (0, 0)),
            hbm, hbm, hbm, hbm, hbm,
        ],
        out_specs=pl.BlockSpec((D, TM), lambda i: (0, jnp.maximum(i - 1, 0))),
        out_shape=jax.ShapeDtypeStruct((D, S), A_x.dtype),
        scratch_shapes=[
            pltpu.VMEM((8, D), f32),
            pltpu.VMEM((TM + _HALO, DP), f32),
            pltpu.VMEM((TM + _HALO, DP), f32),
            pltpu.VMEM((TM, DP), f32),
            pltpu.VMEM((TM, D), f32),
            pltpu.VMEM((TM, D), bf16),
            pltpu.VMEM((TM, D), f32),
            pltpu.VMEM((TM, D), f32),
            pltpu.VMEM((TM, D), bf16),
            pltpu.VMEM((TM, D), f32),
            pltpu.VMEM((D, 3 * D), bf16),
            pltpu.VMEM((D, D), bf16),
            pltpu.VMEM((D, 6 * D), bf16),
            pltpu.VMEM((D, DP), bf16),
            pltpu.VMEM((D, DP), bf16),
            pltpu.VMEM((D, DP), bf16),
            pltpu.VMEM((DP, D), bf16),
            pltpu.VMEM((D, Dff), bf16),
            pltpu.VMEM((D, Dff), bf16),
            pltpu.SemaphoreType.DMA((3 + 2 * (NH + 1),)),
        ],
        compiler_params=pltpu.CompilerParams(
            dimension_semantics=("arbitrary",),
            vmem_limit_bytes=100 * 1024 * 1024,
        ),
    )(x, c, A_wqkv, A_wo, B_w1, w2t, w_mod)
    return out.T.reshape(B, S, D)
```
